```python
import jax
import jax.numpy as jnp

def _softmax(x, axis=-1):
    return jax.nn.softmax(x, axis=axis)
def _gelu(x):
    return jax.nn.gelu(x, approximate=True)
def _silu(x):
    return jax.nn.silu(x)
def _sigmoid(x):
    return jax.nn.sigmoid(x)
def _layernorm(x, axis=-1, eps=1e-5):
    m = jnp.mean(x, axis=axis, keepdims=True)
    v = jnp.var(x, axis=axis, keepdims=True)
    return (x - m) / jnp.sqrt(v + eps)
def _scatter_add(tgt, idx, src, axis=0):
    return tgt.at[idx].add(src)
def _segment_sum(src, seg, n):
    return jax.ops.segment_sum(src, seg, n)
class _Rng:
    def __init__(self, key):
        self._k = key
    def _next(self):
        self._k, sub = jax.random.split(self._k)
        return sub
    def normal(self, shape):
        return jax.random.normal(self._next(), shape, dtype=jnp.bfloat16)
    def randint(self, lo, hi, shape):
        return jax.random.randint(self._next(), shape, lo, hi, dtype=jnp.int32)
    def uniform(self, shape, lo=0.0, hi=1.0):
        return jax.random.uniform(self._next(), shape, jnp.bfloat16, lo, hi)
    def permutation(self, n):
        return jax.random.permutation(self._next(), n)


kernel_name = 'concat_heads__gqa_block_cached__gqa_block_cached__near_ridge'

def setup_inputs():
    _rng = _Rng(jax.random.key(int.from_bytes(__import__("os").urandom(4), "little")))
    _w = (lambda a: (lambda t: t.astype(jnp.bfloat16) if jnp.issubdtype(t.dtype, jnp.floating) else t)(jnp.asarray(a)))
    def _A_setup():
        B, Sq, D = 8, 256, 640
        Hq, Hkv, Sk, Dh = 32, 32, 1024, 192
        assert Hq % Hkv == 0, (Hq, Hkv)
        return {
            "x": _w((lambda *s: _rng.normal(s) * 0.05)(B, Sq, D)),
            "k_cache": _w((lambda *s: _rng.normal(s) * 0.05)(B, Hkv, Sk, Dh)),
            "v_cache": _w((lambda *s: _rng.normal(s) * 0.05)(B, Hkv, Sk, Dh)),
            "wq": _w((lambda *s: _rng.normal(s) * 0.05)(D, Hq * Dh) * (D ** -0.5)),
            "wo": _w((lambda *s: _rng.normal(s) * 0.05)(Hq * Dh, D) * ((Hq * Dh) ** -0.5)),
        }
    _A_in = _A_setup()

    def _B_setup():
        B, Sq, D = 8, 256, 640
        Hq, Hkv, Sk, Dh = 32, 32, 1024, 192
        assert Hq % Hkv == 0, (Hq, Hkv)
        return {
            "x": _w((lambda *s: _rng.normal(s) * 0.05)(B, Sq, D)),
            "k_cache": _w((lambda *s: _rng.normal(s) * 0.05)(B, Hkv, Sk, Dh)),
            "v_cache": _w((lambda *s: _rng.normal(s) * 0.05)(B, Hkv, Sk, Dh)),
            "wq": _w((lambda *s: _rng.normal(s) * 0.05)(D, Hq * Dh) * (D ** -0.5)),
            "wo": _w((lambda *s: _rng.normal(s) * 0.05)(Hq * Dh, D) * ((Hq * Dh) ** -0.5)),
        }
    _B_in = _B_setup()

    return {
        "A_x": _A_in["x"],
        "A_k_cache": _A_in["k_cache"],
        "A_v_cache": _A_in["v_cache"],
        "A_wq": _A_in["wq"],
        "A_wo": _A_in["wo"],
        "B_x": _B_in["x"],
        "B_k_cache": _B_in["k_cache"],
        "B_v_cache": _B_in["v_cache"],
        "B_wq": _B_in["wq"],
        "B_wo": _B_in["wo"],
    }

def reference(A_x, A_k_cache, A_v_cache, A_wq, A_wo, B_x, B_k_cache, B_v_cache, B_wq, B_wo):
    def _A_ref(x, k_cache, v_cache, wq, wo):
        B, Sq, D = x.shape
        Hq, Dh = 32, 192
        Hkv = k_cache.shape[1]
        rep = Hq // Hkv
        q = (lambda x, *d: x.transpose(*d))((x @ wq).reshape(B, Sq, Hq, Dh), 0, 2, 1, 3)
        k = jnp.repeat(k_cache, rep, axis=1)
        v = jnp.repeat(v_cache, rep, axis=1)
        scores = jnp.einsum("bhqd,bhkd->bhqk", q, k) * (Dh ** -0.5)
        p = _softmax(scores, axis=-1)
        o = jnp.einsum("bhqk,bhkd->bhqd", p, v)
        return (lambda x, *d: x.transpose(*d))(o, 0, 2, 1, 3).reshape(B, Sq, Hq * Dh) @ wo

    def _B_ref(x, k_cache, v_cache, wq, wo):
        B, Sq, D = x.shape
        Hq, Dh = 32, 192
        Hkv = k_cache.shape[1]
        rep = Hq // Hkv
        q = (lambda x, *d: x.transpose(*d))((x @ wq).reshape(B, Sq, Hq, Dh), 0, 2, 1, 3)
        k = jnp.repeat(k_cache, rep, axis=1)
        v = jnp.repeat(v_cache, rep, axis=1)
        scores = jnp.einsum("bhqd,bhkd->bhqk", q, k) * (Dh ** -0.5)
        p = _softmax(scores, axis=-1)
        o = jnp.einsum("bhqk,bhkd->bhqd", p, v)
        return (lambda x, *d: x.transpose(*d))(o, 0, 2, 1, 3).reshape(B, Sq, Hq * Dh) @ wo

    a = _A_ref(A_x, A_k_cache, A_v_cache, A_wq, A_wo)
    b = _B_ref(B_x, B_k_cache, B_v_cache, B_wq, B_wo)
    return jnp.concatenate([a, b], axis=-1)
```

```python
import jax
import jax.numpy as jnp
from jax.experimental import pallas as pl
from jax.experimental.pallas import tpu as pltpu

_LOG2E = 1.4426950408889634
_NT = (((1,), (1,)), ((), ()))
_F32 = jnp.float32
_BF16 = jnp.bfloat16


def _qproj(x, wq_ref, hp, dh):
    q = jnp.dot(x, wq_ref[:, hp * 2 * dh:(hp + 1) * 2 * dh], preferred_element_type=_F32)
    return (q * (dh ** -0.5 * _LOG2E)).astype(_BF16)


def _scores(q, j, kt_ref, h, dh):
    return jnp.dot(q[:, j * dh:(j + 1) * dh], kt_ref[0, h], preferred_element_type=_F32)


def _softmax_parts(s):
    m = jnp.max(s, axis=-1, keepdims=True)
    p = jnp.exp2(s - m)
    l = jnp.sum(p, axis=-1, keepdims=True)
    return p.astype(_BF16), 1.0 / l


def _pv_t(p, vt_ref, h):
    return jax.lax.dot_general(vt_ref[0, h], p, _NT, preferred_element_type=_F32)


def _out_proj(ot0, ot1, li0, li1, wo_ref, hp, dh):
    sq = ot0.shape[1]
    o = jnp.concatenate([ot0, ot1], axis=0).T
    li = jnp.concatenate(
        [jnp.broadcast_to(li0, (sq, dh)), jnp.broadcast_to(li1, (sq, dh))], axis=1)
    o = (o * li).astype(_BF16)
    return jnp.dot(o, wo_ref[hp * 2 * dh:(hp + 1) * 2 * dh, :], preferred_element_type=_F32)


@jax.jit
def pallas_concat_heads__gqa_block_cached__gqa_block_cached__near_ridge_kernel(
    A_x, A_k_cache, A_v_cache, A_wq, A_wo, B_x, B_k_cache, B_v_cache, B_wq, B_wo,
):
    B, SQ, D = A_x.shape
    _, H, SK, DH = A_k_cache.shape
    hb = 4
    HG = H // hb

    def kern(xa, ka, va, wqa, woa, xb, kb, vb, wqb, wob, o_ref, acca, accb):
        g = pl.program_id(0)
        b = pl.program_id(1)

        @pl.when(g == 0)
        def _():
            acca[b] = jnp.zeros((SQ, D), _F32)
            accb[b] = jnp.zeros((SQ, D), _F32)

        x_a = xa[0]
        x_b = xb[0]
        for hp in range(hb // 2):
            h0 = 2 * hp
            h1 = h0 + 1
            qa = _qproj(x_a, wqa, hp, DH)
            qb = _qproj(x_b, wqb, hp, DH)
            sa0 = _scores(qa, 0, ka, h0, DH)
            sa1 = _scores(qa, 1, ka, h1, DH)
            pa0, la0 = _softmax_parts(sa0)
            sb0 = _scores(qb, 0, kb, h0, DH)
            pa1, la1 = _softmax_parts(sa1)
            oa0 = _pv_t(pa0, va, h0)
            sb1 = _scores(qb, 1, kb, h1, DH)
            pb0, lb0 = _softmax_parts(sb0)
            oa1 = _pv_t(pa1, va, h1)
            pb1, lb1 = _softmax_parts(sb1)
            ob0 = _pv_t(pb0, vb, h0)
            ob1 = _pv_t(pb1, vb, h1)
            acca[b] += _out_proj(oa0, oa1, la0, la1, woa, hp, DH)
            accb[b] += _out_proj(ob0, ob1, lb0, lb1, wob, hp, DH)

        @pl.when(g == HG - 1)
        def _():
            o_ref[0, :, 0:D] = acca[b].astype(_BF16)
            o_ref[0, :, D:2 * D] = accb[b].astype(_BF16)

    t = lambda a: a.transpose(0, 1, 3, 2)
    xs = pl.BlockSpec((1, SQ, D), lambda g, b: (b, 0, 0))
    ks = pl.BlockSpec((1, hb, DH, SK), lambda g, b: (b, g, 0, 0))
    wqs = pl.BlockSpec((D, hb * DH), lambda g, b: (0, g))
    wos = pl.BlockSpec((hb * DH, D), lambda g, b: (g, 0))
    return pl.pallas_call(
        kern,
        grid=(HG, B),
        in_specs=[xs, ks, ks, wqs, wos] * 2,
        out_specs=pl.BlockSpec((1, SQ, 2 * D), lambda g, b: (jnp.where(g == HG - 1, b, 0), 0, 0)),
        out_shape=jax.ShapeDtypeStruct((B, SQ, 2 * D), _BF16),
        scratch_shapes=[pltpu.VMEM((B, SQ, D), _F32)] * 2,
        compiler_params=pltpu.CompilerParams(
            dimension_semantics=("arbitrary", "arbitrary"), vmem_limit_bytes=100 * 2**20),
    )(A_x, t(A_k_cache), t(A_v_cache), A_wq, A_wo, B_x, t(B_k_cache), t(B_v_cache), B_wq, B_wo)
```

```python
import jax, jax.numpy as jnp
from jax import lax
from jax.experimental import pallas as pl
from jax.experimental.pallas import tpu as pltpu

B,SQ,D,H,SK,DH = 8,256,640,32,1024,192
LOG2E = 1.4426950408889634
NT = (((1,),(1,)),((),()))
f32=jnp.float32; bf=jnp.bfloat16
DEF = "qb qa sb0 sa0 mb0 sa1 pb0 ma0 sb1 ma1 pa0 mb1 pa1 pb1 oa ob"

def make(hb=2, order=DEF, vmem=100):
    G = H//hb; T = G*B; W = hb*DH
    order = order.split()
    def kern(xa,ka,va,wqa,woa, xb,kb,vb,wqb,wob, o_hbm,
             xbuf, kbuf, vbuf, wqbuf, wobuf, acc, obuf, sem_x, sem_kv, sem_w, sem_o):
        xs=(xa,xb); ks=(ka,kb); vs=(va,vb); wqs=(wqa,wqb); wos=(woa,wob)
        def kv_copies(t, slot):
            g = t >> 3; b = t & 7
            cs=[]
            for br in range(2):
                cs.append(pltpu.make_async_copy(ks[br].at[b, pl.ds(g*hb, hb)], kbuf.at[slot, br], sem_kv.at[slot, 0, br]))
            for br in range(2):
                cs.append(pltpu.make_async_copy(vs[br].at[b, pl.ds(g*hb, hb)], vbuf.at[slot, br], sem_kv.at[slot, 1, br]))
            return cs
        def w_copies(g, slot):
            cs=[]
            for br in range(2):
                cs.append(pltpu.make_async_copy(wqs[br].at[:, pl.ds(pl.multiple_of(g*W, W), W)], wqbuf.at[slot, br], sem_w.at[slot, 0, br]))
            for br in range(2):
                cs.append(pltpu.make_async_copy(wos[br].at[pl.ds(pl.multiple_of(g*W, W), W), :], wobuf.at[slot, br], sem_w.at[slot, 1, br]))
            return cs
        xc0 = [pltpu.make_async_copy(xs[br].at[pl.ds(0,1)], xbuf.at[br, pl.ds(0,1)], sem_x.at[br]) for br in range(2)]
        xc1 = [pltpu.make_async_copy(xs[br].at[pl.ds(1,B-1)], xbuf.at[br, pl.ds(1,B-1)], sem_x.at[2+br]) for br in range(2)]
        w0 = w_copies(0, 0)
        w0[0].start(); xc0[0].start(); w0[1].start(); xc0[1].start()
        kv0 = kv_copies(0, 0)
        for c in kv0: c.start()
        w0[2].start(); w0[3].start()
        acc[...] = jnp.zeros(acc.shape, f32)
        for c in xc0: c.wait()
        for c in kv0: c.wait()
        for c in kv_copies(1, 1): c.start()
        for c in xc1: c.start()
        def emit(b):
            obuf[b, :, 0:D] = acc[0,b].astype(bf)
            obuf[b, :, D:2*D] = acc[1,b].astype(bf)
            pltpu.make_async_copy(obuf.at[b], o_hbm.at[b], sem_o.at[b]).start()
        def step(t, carry):
            g = t >> 3; b = t & 7
            slot = t & 1; ws = g & 1
            @pl.when(b == 0)
            def _():
                for c in w_copies(g, ws): c.wait()
            @pl.when(t == 1)
            def _():
                for c in xc1: c.wait()
            @pl.when(t > 0)
            def _():
                for c in kv_copies(t, slot): c.wait()
            @pl.when(t > T-B)
            def _():
                emit(b-1)
            for hp in range(hb//2):
                cs=slice(hp*384,(hp+1)*384)
                st={}
                for op in order:
                    k=op[0]; br="ab".index(op[1])
                    if k=="q":
                        q = jnp.dot(xbuf[br,b], wqbuf[ws,br,:,cs], preferred_element_type=f32)
                        st[op] = (q * (DH**-0.5*LOG2E)).astype(bf)
                    elif k=="s":
                        j=int(op[2])
                        st[op] = jnp.dot(st["q"+op[1]][:, j*192:(j+1)*192], kbuf[slot,br,2*hp+j], preferred_element_type=f32)
                    elif k=="m":
                        s = st.pop("s"+op[1:])
                        m = jnp.max(s, axis=-1, keepdims=True)
                        p = jnp.exp2(s-m)
                        l = jnp.sum(p, axis=-1, keepdims=True)
                        st[op] = (p.astype(bf), 1.0/l)
                    elif k=="p":
                        j=int(op[2])
                        p,li = st.pop("m"+op[1:])
                        ot = lax.dot_general(vbuf[slot,br,2*hp+j], p, NT, preferred_element_type=f32)
                        st[op] = (ot, li)
                    elif k=="o":
                        (o0,l0),(o1,l1) = st.pop("p"+op[1]+"0"), st.pop("p"+op[1]+"1")
                        o = jnp.concatenate([o0, o1], axis=0).T
                        li = jnp.concatenate([jnp.broadcast_to(l0,(256,192)), jnp.broadcast_to(l1,(256,192))],axis=1)
                        o = (o*li).astype(bf)
                        acc[br,b] += jnp.dot(o, wobuf[ws,br,cs,:], preferred_element_type=f32)
            @pl.when(t+2 < T)
            def _():
                for c in kv_copies(t+2, slot): c.start()
            @pl.when((b == 0) & (g+1 < G))
            def _():
                for c in w_copies(g+1, 1-ws): c.start()
            return carry
        lax.fori_loop(0, T, step, 0)
        emit(B-1)
        for b in range(B):
            pltpu.make_async_copy(obuf.at[b], o_hbm.at[b], sem_o.at[b]).wait()

    def fn(xa,ka,va,wqa,woa, xb,kb,vb,wqb,wob):
        t = lambda a: a.transpose(0,1,3,2)
        anyspec = pl.BlockSpec(memory_space=pl.ANY)
        return pl.pallas_call(kern,
            in_specs=[anyspec]*10, out_specs=anyspec,
            out_shape=jax.ShapeDtypeStruct((B,SQ,2*D), bf),
            scratch_shapes=[pltpu.VMEM((2,B,SQ,D),bf), pltpu.VMEM((2,2,hb,DH,SK),bf), pltpu.VMEM((2,2,hb,DH,SK),bf),
                            pltpu.VMEM((2,2,D,W),bf), pltpu.VMEM((2,2,W,D),bf), pltpu.VMEM((2,B,SQ,D),f32), pltpu.VMEM((B,SQ,2*D),bf),
                            pltpu.SemaphoreType.DMA((4,)), pltpu.SemaphoreType.DMA((2,2,2)), pltpu.SemaphoreType.DMA((2,2,2)), pltpu.SemaphoreType.DMA((B,))],
            compiler_params=pltpu.CompilerParams(vmem_limit_bytes=vmem*2**20, disable_bounds_checks=True),
        )(xa,t(ka),t(va),wqa,woa, xb,t(kb),t(vb),wqb,wob)
    return fn


@jax.jit
def pallas_concat_heads__gqa_block_cached__gqa_block_cached__near_ridge_kernel(A_x, A_k_cache, A_v_cache, A_wq, A_wo, B_x, B_k_cache, B_v_cache, B_wq, B_wo):
    return make()(A_x, A_k_cache, A_v_cache, A_wq, A_wo, B_x, B_k_cache, B_v_cache, B_wq, B_wo)
```
